```python
import os as _os
_os.environ.setdefault("JAX_PLATFORMS", "cpu")
import jax
import jax.numpy as jnp

def _softmax(x, axis=-1):
    return jax.nn.softmax(x, axis=axis)
def _gelu(x):
    return jax.nn.gelu(x, approximate=True)
def _silu(x):
    return jax.nn.silu(x)
def _sigmoid(x):
    return jax.nn.sigmoid(x)
def _layernorm(x, axis=-1, eps=1e-5):
    m = jnp.mean(x, axis=axis, keepdims=True)
    v = jnp.var(x, axis=axis, keepdims=True)
    return (x - m) / jnp.sqrt(v + eps)
def _scatter_add(tgt, idx, src, axis=0):
    return tgt.at[idx].add(src)
def _segment_sum(src, seg, n):
    return jax.ops.segment_sum(src, seg, n)
class _Rng:
    def __init__(self, key):
        self._k = key
    def _next(self):
        self._k, sub = jax.random.split(self._k)
        return sub
    def normal(self, shape):
        return jax.random.normal(self._next(), shape, dtype=jnp.bfloat16)
    def randint(self, lo, hi, shape):
        return jax.random.randint(self._next(), shape, lo, hi, dtype=jnp.int32)
    def uniform(self, shape, lo=0.0, hi=1.0):
        return jax.random.uniform(self._next(), shape, jnp.bfloat16, lo, hi)
    def permutation(self, n):
        return jax.random.permutation(self._next(), n)


kernel_name = 'standalone__linear_kernel_rfa__decode'

def setup_inputs():
    _rng = _Rng(jax.random.key(int.from_bytes(__import__("os").urandom(4), "little")))
    _w = (lambda a: (lambda t: t.astype(jnp.bfloat16) if jnp.issubdtype(t.dtype, jnp.floating) else t)(jnp.asarray(a)))
    B, H, Sq, Sk, D, M = 2, 16, 1, 16384, 256, 16
    return {
        "q": _w((lambda *s: _rng.normal(s) * 0.4)(B, H, Sq, D)),
        "k": _w((lambda *s: _rng.normal(s) * 1.6)(B, H, Sk, D)),
        "v": _w((lambda *s: _rng.normal(s) * 1.6)(B, H, Sk, D)),
        "omega": _w((lambda *s: _rng.normal(s) * 1.6)(M, D)),
    }

def reference(q, k, v, omega):
    d = q.shape[-1]
    m = omega.shape[0]
    scale = float(d) ** -0.25
    qs = q * scale
    ks = k * scale
    q_proj = jnp.einsum("bhsd,md->bhsm", qs, omega)
    k_proj = jnp.einsum("bhsd,md->bhsm", ks, omega)
    q_sq = 0.5 * jnp.einsum("bhsd,bhsd->bhs", qs, qs)[..., None]
    k_sq = 0.5 * jnp.einsum("bhsd,bhsd->bhs", ks, ks)[..., None]
    inv_sqrt_m = float(m) ** -0.5
    phi_q = jnp.exp(q_proj - q_sq) * inv_sqrt_m + 1e-6
    phi_k = jnp.exp(k_proj - k_sq) * inv_sqrt_m + 1e-6
    kv = jnp.einsum("bhsm,bhsd->bhmd", phi_k, v)
    z  = jnp.einsum("bhsm->bhm", phi_k)
    num = jnp.einsum("bhqm,bhmd->bhqd", phi_q, kv)
    den = jnp.einsum("bhqm,bhm->bhq", phi_q, z)[..., None] + 1e-6
    return num / den
```

```python
import functools

import jax
import jax.numpy as jnp
import jax.experimental.pallas as pl
import jax.experimental.pallas.tpu as pltpu

_DMA_ROWS = 64
_STREAMS = 8
_STEP_ROWS = 1024
_NBUF = 5
_LANES = 128


def _rfa_kernel(q_ref, k_hbm, v_hbm, om_ref, o_ref, kb, vb, sems, qs_scr, out_scr,
                *, scale, inv_sqrt_m, sk):
    M, D = om_ref.shape
    T, C, NS, NBUF = _DMA_ROWS, _STEP_ROWS, _STREAMS, _NBUF
    n_heads = q_ref.shape[0]
    steps_per_head = sk // C
    n_steps = n_heads * steps_per_head
    stream_len = sk // NS

    def start(i):
        slot = jax.lax.rem(i, NBUF)
        base = (i // steps_per_head) * sk + jax.lax.rem(i, steps_per_head) * (C // NS)
        for g in range(C // T):
            r = pl.multiple_of(base + (g % NS) * stream_len + (g // NS) * T, T)
            pltpu.make_async_copy(k_hbm.at[pl.ds(r, T)], kb.at[slot, pl.ds(g * T, T)],
                                  sems.at[0, slot]).start(priority=0)
            pltpu.make_async_copy(v_hbm.at[pl.ds(r, T)], vb.at[slot, pl.ds(g * T, T)],
                                  sems.at[1, slot]).start(priority=1)

    for i in range(NBUF - 1):
        start(i)

    omf = om_ref[...].astype(jnp.float32)
    lhs = jnp.concatenate(
        [(omf * scale).astype(jnp.bfloat16),
         jnp.full((M, _LANES), -0.5 * scale * scale, jnp.bfloat16)], axis=1)
    qs_scr[...] = q_ref[...].astype(jnp.float32) * scale

    def head(bh, _):
        def step(j, carry):
            kv, z = carry
            i = bh * steps_per_head + j
            slot = jax.lax.rem(i, NBUF)

            @pl.when(i + NBUF - 1 < n_steps)
            def _():
                start(i + NBUF - 1)

            pltpu.make_async_copy(kb.at[slot], kb.at[slot], sems.at[0, slot]).wait()
            pltpu.make_async_copy(vb.at[slot], vb.at[slot], sems.at[1, slot]).wait()

            kc = kb[slot]
            kf = kc.astype(jnp.float32)
            sq = kf[:, :_LANES] * kf[:, :_LANES]
            for t in range(1, D // _LANES):
                blk = kf[:, t * _LANES:(t + 1) * _LANES]
                sq = sq + blk * blk
            rhs = jnp.concatenate([kc, sq.astype(jnp.bfloat16)], axis=1)
            logits = jax.lax.dot_general(
                lhs, rhs, (((1,), (1,)), ((), ())),
                preferred_element_type=jnp.float32)
            phi = (jnp.exp(logits) * inv_sqrt_m + 1e-6).astype(jnp.bfloat16)
            kv = kv + jnp.dot(phi, vb[slot], preferred_element_type=jnp.float32)
            pf = phi.astype(jnp.float32)
            for t in range(C // _LANES):
                z = z + pf[:, t * _LANES:(t + 1) * _LANES]
            return kv, z

        kv, z = jax.lax.fori_loop(
            0, steps_per_head, step,
            (jnp.zeros((M, D), jnp.float32), jnp.zeros((M, _LANES), jnp.float32)))

        qs = qs_scr[pl.ds(bh, 1), :]
        q_proj = jnp.sum(omf * qs, axis=1, keepdims=True)
        q_sq = 0.5 * jnp.sum(qs * qs, axis=1, keepdims=True)
        phi_q = jnp.exp(q_proj - q_sq) * inv_sqrt_m + 1e-6
        num = jnp.sum(phi_q * kv, axis=0, keepdims=True)
        den = jnp.sum(phi_q * jnp.sum(z, axis=1, keepdims=True),
                      axis=0, keepdims=True) + 1e-6
        out_scr[pl.ds(bh, 1), :] = num / den
        return 0

    jax.lax.fori_loop(0, n_heads, head, 0)
    o_ref[...] = out_scr[...].astype(o_ref.dtype)


@jax.jit
def pallas_standalone__linear_kernel_rfa__decode_kernel(
    q: jax.Array,
    k: jax.Array,
    v: jax.Array,
    omega: jax.Array,
):
    B, H, Sq, D = q.shape
    Sk = k.shape[2]
    M = omega.shape[0]
    assert Sq == 1 and D % _LANES == 0
    assert Sk % _STEP_ROWS == 0 and _STEP_ROWS % (_STREAMS * _DMA_ROWS) == 0
    assert B * H * (Sk // _STEP_ROWS) >= _NBUF - 1

    out = pl.pallas_call(
        functools.partial(_rfa_kernel, scale=float(D) ** -0.25,
                          inv_sqrt_m=float(M) ** -0.5, sk=Sk),
        in_specs=[
            pl.BlockSpec(memory_space=pltpu.VMEM),
            pl.BlockSpec(memory_space=pl.ANY),
            pl.BlockSpec(memory_space=pl.ANY),
            pl.BlockSpec(memory_space=pltpu.VMEM),
        ],
        out_specs=pl.BlockSpec(memory_space=pltpu.VMEM),
        out_shape=jax.ShapeDtypeStruct((B * H, D), q.dtype),
        scratch_shapes=[
            pltpu.VMEM((_NBUF, _STEP_ROWS, D), k.dtype),
            pltpu.VMEM((_NBUF, _STEP_ROWS, D), v.dtype),
            pltpu.SemaphoreType.DMA((2, _NBUF)),
            pltpu.VMEM((B * H, D), jnp.float32),
            pltpu.VMEM((B * H, D), jnp.float32),
        ],
        compiler_params=pltpu.CompilerParams(vmem_limit_bytes=32 * 1024 * 1024),
    )(q.reshape(B * H, D), k.reshape(B * H * Sk, D), v.reshape(B * H * Sk, D), omega)
    return out.reshape(B, H, Sq, D)
```
